```python
import os as _os
_os.environ.setdefault("JAX_PLATFORMS", "cpu")
import jax
import jax.numpy as jnp

def _softmax(x, axis=-1):
    return jax.nn.softmax(x, axis=axis)
def _gelu(x):
    return jax.nn.gelu(x, approximate=True)
def _silu(x):
    return jax.nn.silu(x)
def _sigmoid(x):
    return jax.nn.sigmoid(x)
def _layernorm(x, axis=-1, eps=1e-5):
    m = jnp.mean(x, axis=axis, keepdims=True)
    v = jnp.var(x, axis=axis, keepdims=True)
    return (x - m) / jnp.sqrt(v + eps)
def _scatter_add(tgt, idx, src, axis=0):
    return tgt.at[idx].add(src)
def _segment_sum(src, seg, n):
    return jax.ops.segment_sum(src, seg, n)
class _Rng:
    def __init__(self, key):
        self._k = key
    def _next(self):
        self._k, sub = jax.random.split(self._k)
        return sub
    def normal(self, shape):
        return jax.random.normal(self._next(), shape, dtype=jnp.bfloat16)
    def randint(self, lo, hi, shape):
        return jax.random.randint(self._next(), shape, lo, hi, dtype=jnp.int32)
    def uniform(self, shape, lo=0.0, hi=1.0):
        return jax.random.uniform(self._next(), shape, jnp.bfloat16, lo, hi)
    def permutation(self, n):
        return jax.random.permutation(self._next(), n)


kernel_name = 'concat_heads__gqa_block_cached__gqa_block_cached__near_ridge'

def setup_inputs():
    _rng = _Rng(jax.random.key(int.from_bytes(__import__("os").urandom(4), "little")))
    _w = (lambda a: (lambda t: t.astype(jnp.bfloat16) if jnp.issubdtype(t.dtype, jnp.floating) else t)(jnp.asarray(a)))
    def _A_setup():
        B, Sq, D = 8, 128, 576
        Hq, Hkv, Sk, Dh = 32, 16, 512, 128
        assert Hq % Hkv == 0, (Hq, Hkv)
        return {
            "x": _w((lambda *s: _rng.normal(s) * 0.8)(B, Sq, D)),
            "k_cache": _w((lambda *s: _rng.normal(s) * 0.8)(B, Hkv, Sk, Dh)),
            "v_cache": _w((lambda *s: _rng.normal(s) * 0.05)(B, Hkv, Sk, Dh)),
            "wq": _w((lambda *s: _rng.normal(s) * 0.8)(D, Hq * Dh) * (D ** -0.5)),
            "wo": _w((lambda *s: _rng.normal(s) * 0.05)(Hq * Dh, D) * ((Hq * Dh) ** -0.5)),
        }
    _A_in = _A_setup()

    def _B_setup():
        B, Sq, D = 8, 128, 576
        Hq, Hkv, Sk, Dh = 32, 16, 512, 128
        assert Hq % Hkv == 0, (Hq, Hkv)
        return {
            "x": _w((lambda *s: _rng.normal(s) * 0.8)(B, Sq, D)),
            "k_cache": _w((lambda *s: _rng.normal(s) * 0.8)(B, Hkv, Sk, Dh)),
            "v_cache": _w((lambda *s: _rng.normal(s) * 0.05)(B, Hkv, Sk, Dh)),
            "wq": _w((lambda *s: _rng.normal(s) * 0.8)(D, Hq * Dh) * (D ** -0.5)),
            "wo": _w((lambda *s: _rng.normal(s) * 0.05)(Hq * Dh, D) * ((Hq * Dh) ** -0.5)),
        }
    _B_in = _B_setup()

    return {
        "A_x": _A_in["x"],
        "A_k_cache": _A_in["k_cache"],
        "A_v_cache": _A_in["v_cache"],
        "A_wq": _A_in["wq"],
        "A_wo": _A_in["wo"],
        "B_x": _B_in["x"],
        "B_k_cache": _B_in["k_cache"],
        "B_v_cache": _B_in["v_cache"],
        "B_wq": _B_in["wq"],
        "B_wo": _B_in["wo"],
    }

def reference(A_x, A_k_cache, A_v_cache, A_wq, A_wo, B_x, B_k_cache, B_v_cache, B_wq, B_wo):
    def _A_ref(x, k_cache, v_cache, wq, wo):
        B, Sq, D = x.shape
        Hq, Dh = 32, 128
        Hkv = k_cache.shape[1]
        rep = Hq // Hkv
        q = (lambda x, *d: x.transpose(*d))((x @ wq).reshape(B, Sq, Hq, Dh), 0, 2, 1, 3)
        k = jnp.repeat(k_cache, rep, axis=1)
        v = jnp.repeat(v_cache, rep, axis=1)
        scores = jnp.einsum("bhqd,bhkd->bhqk", q, k) * (Dh ** -0.5)
        p = _softmax(scores, axis=-1)
        o = jnp.einsum("bhqk,bhkd->bhqd", p, v)
        return (lambda x, *d: x.transpose(*d))(o, 0, 2, 1, 3).reshape(B, Sq, Hq * Dh) @ wo

    def _B_ref(x, k_cache, v_cache, wq, wo):
        B, Sq, D = x.shape
        Hq, Dh = 32, 128
        Hkv = k_cache.shape[1]
        rep = Hq // Hkv
        q = (lambda x, *d: x.transpose(*d))((x @ wq).reshape(B, Sq, Hq, Dh), 0, 2, 1, 3)
        k = jnp.repeat(k_cache, rep, axis=1)
        v = jnp.repeat(v_cache, rep, axis=1)
        scores = jnp.einsum("bhqd,bhkd->bhqk", q, k) * (Dh ** -0.5)
        p = _softmax(scores, axis=-1)
        o = jnp.einsum("bhqk,bhkd->bhqd", p, v)
        return (lambda x, *d: x.transpose(*d))(o, 0, 2, 1, 3).reshape(B, Sq, Hq * Dh) @ wo

    a = _A_ref(A_x, A_k_cache, A_v_cache, A_wq, A_wo)
    b = _B_ref(B_x, B_k_cache, B_v_cache, B_wq, B_wo)
    return jnp.concatenate([a, b], axis=-1)
```

```python
import functools
import math
import jax
import jax.numpy as jnp
from jax import lax
import jax.experimental.pallas as pl
import jax.experimental.pallas.tpu as pltpu

B, SQ, D = 8, 128, 576
HQ, HKV, SK, DH = 32, 16, 512, 128
REP = HQ // HKV
GW = REP * DH
M = B * SQ
QSCALE = (DH ** -0.5) * math.log2(math.e)
CB = 2
HPS = 2
BPS = 4
NBH = B // BPS
NC = BPS // CB
SPP = (HKV // HPS) * NBH
NSTEP = 2 * SPP
W = HPS * GW
OCH = 4


def _kernel(axt, ak, av, awq, awot, bxt, bk, bv, bwq, bwot, out_hbm,
            kbuf, vbuf, wqbuf, wobuf, xtbuf, x_ref, acc_ref, outbuf,
            sem_kv, sem_w, sem_misc, sem_out):
    s = pl.program_id(0)
    ph = s // SPP
    t = s % SPP
    hp = t // NBH
    bh = t % NBH
    slot = s % 2
    wslot = (s // NBH) % 2

    def w_copies(wq_hbm, wo_hbm, hh, sl):
        cols = pl.ds(pl.multiple_of(hh * W, W), W)
        return (pltpu.make_async_copy(wq_hbm.at[:, cols], wqbuf.at[sl], sem_w.at[0, sl]),
                pltpu.make_async_copy(wo_hbm.at[:, cols], wobuf.at[sl], sem_w.at[1, sl]))

    def kv_copies(k_hbm, v_hbm, hh, bb, sl):
        heads = pl.ds(hh * HPS, HPS)
        bs = pl.ds(bb * BPS, BPS)
        return (pltpu.make_async_copy(k_hbm.at[bs, heads], kbuf.at[sl], sem_kv.at[0, sl]),
                pltpu.make_async_copy(v_hbm.at[bs, heads], vbuf.at[sl], sem_kv.at[1, sl]))

    @pl.when(s == 0)
    def _():
        pltpu.make_async_copy(axt, xtbuf, sem_misc.at[0]).start()
        wc = w_copies(awq, awot, 0, 0)
        wc[0].start()
        for cp in kv_copies(ak, av, 0, 0, 0):
            cp.start()
        wc[1].start()

    @pl.when(t == 0)
    def _():
        acc_ref[...] = jnp.zeros_like(acc_ref)
        pltpu.make_async_copy(axt, xtbuf, sem_misc.at[0]).wait()
        for b in range(B):
            x_ref[b * SQ:(b + 1) * SQ, :] = xtbuf[b].T

    @pl.when(bh == 0)
    def _():
        for cp in w_copies(awq, awot, 0, wslot):
            cp.wait()

    for cp in kv_copies(ak, av, 0, 0, slot):
        cp.wait()

    nxt = s + 1
    nt = nxt % SPP
    nhp = nt // NBH
    nbh = nt % NBH

    @pl.when(nxt < SPP)
    def _():
        for cp in kv_copies(ak, av, nhp, nbh, 1 - slot):
            cp.start()

        @pl.when(nbh == 0)
        def _():
            for cp in w_copies(awq, awot, nhp, 1 - wslot):
                cp.start()

    @pl.when(jnp.logical_and(nxt >= SPP, nxt < NSTEP))
    def _():
        for cp in kv_copies(bk, bv, nhp, nbh, 1 - slot):
            cp.start()

        @pl.when(nbh == 0)
        def _():
            for cp in w_copies(bwq, bwot, nhp, 1 - wslot):
                cp.start()

    @pl.when(s == 1)
    def _():
        pltpu.make_async_copy(bxt, xtbuf, sem_misc.at[0]).start()

    for c in range(NC):
        r0 = pl.multiple_of(bh * (BPS * SQ) + c * CB * SQ, CB * SQ)
        rows = pl.ds(r0, CB * SQ)
        q = jnp.dot(x_ref[rows, :], wqbuf[wslot], preferred_element_type=jnp.float32)
        q = (q * QSCALE).astype(jnp.bfloat16)
        o_rows = []
        for j in range(CB):
            b = c * CB + j
            o_heads = []
            for g in range(HPS):
                qb = q[j * SQ:(j + 1) * SQ, g * GW:(g + 1) * GW]
                q2 = jnp.concatenate([qb[:, :DH], qb[:, DH:]], axis=0)
                k = kbuf[slot, b, g]
                v = vbuf[slot, b, g]
                sc = lax.dot_general(q2, k, (((1,), (1,)), ((), ())),
                                     preferred_element_type=jnp.float32)
                m = jnp.max(sc, axis=-1, keepdims=True)
                p = jnp.exp2(sc - m)
                l = jnp.sum(p, axis=-1, keepdims=True)
                o2 = jnp.dot(p.astype(jnp.bfloat16), v, preferred_element_type=jnp.float32)
                r = pl.reciprocal(l, approx=True)
                r = r * (2.0 - l * r)
                o2 = (o2 * r).astype(jnp.bfloat16)
                o_heads += [o2[:SQ], o2[SQ:]]
            o_rows.append(jnp.concatenate(o_heads, axis=1))
        o = jnp.concatenate(o_rows, axis=0)
        acc_ref[rows, :] += lax.dot_general(o, wobuf[wslot], (((1,), (1,)), ((), ())),
                                            preferred_element_type=jnp.float32)

    @pl.when(s == SPP - 1)
    def _():
        outbuf[:, 0:D] = acc_ref[...].astype(outbuf.dtype)

    @pl.when(s == NSTEP - 1)
    def _():
        oc = M // OCH
        cps = []
        for c in range(OCH):
            rows = slice(c * oc, (c + 1) * oc)
            outbuf[rows, D:2 * D] = acc_ref[rows, :].astype(outbuf.dtype)
            cp = pltpu.make_async_copy(outbuf.at[rows], out_hbm.at[rows], sem_out.at[c])
            cp.start()
            cps.append(cp)
        for cp in cps:
            cp.wait()


@jax.jit
def pallas_concat_heads__gqa_block_cached__gqa_block_cached__near_ridge_kernel(
    A_x, A_k_cache, A_v_cache, A_wq, A_wo, B_x, B_k_cache, B_v_cache, B_wq, B_wo):
    axt = jnp.swapaxes(A_x, 1, 2)
    bxt = jnp.swapaxes(B_x, 1, 2)
    awot = A_wo.T
    bwot = B_wo.T
    any_spec = pl.BlockSpec(memory_space=pl.ANY)
    out = pl.pallas_call(
        _kernel,
        grid=(NSTEP,),
        in_specs=[any_spec] * 10,
        out_specs=any_spec,
        out_shape=jax.ShapeDtypeStruct((M, 2 * D), jnp.bfloat16),
        scratch_shapes=[
            pltpu.VMEM((2, BPS, HPS, SK, DH), jnp.bfloat16),
            pltpu.VMEM((2, BPS, HPS, SK, DH), jnp.bfloat16),
            pltpu.VMEM((2, D, W), jnp.bfloat16),
            pltpu.VMEM((2, D, W), jnp.bfloat16),
            pltpu.VMEM((B, D, SQ), jnp.bfloat16),
            pltpu.VMEM((M, D), jnp.bfloat16),
            pltpu.VMEM((M, D), jnp.float32),
            pltpu.VMEM((M, 2 * D), jnp.bfloat16),
            pltpu.SemaphoreType.DMA((2, 2)),
            pltpu.SemaphoreType.DMA((2, 2)),
            pltpu.SemaphoreType.DMA((1,)),
            pltpu.SemaphoreType.DMA((OCH,)),
        ],
        compiler_params=pltpu.CompilerParams(
            dimension_semantics=("arbitrary",),
            vmem_limit_bytes=96 * 1024 * 1024,
        ),
    )(axt, A_k_cache, A_v_cache, A_wq, awot, bxt, B_k_cache, B_v_cache, B_wq, bwot)
    return out.reshape(B, SQ, 2 * D)
```

```python
import math

import jax
import jax.numpy as jnp
from jax import lax
import jax.experimental.pallas as pl
import jax.experimental.pallas.tpu as pltpu

B, SQ, D = 8, 128, 576
HQ, HKV, SK, DH = 32, 16, 512, 128
REP = HQ // HKV
GW = REP * DH
M = B * SQ
QSCALE = (DH ** -0.5) * math.log2(math.e)
CB = 2
NC = B // CB
HPS = 2
SPP = HKV // HPS
NSTEP = 2 * SPP
W = HPS * GW

_NT = (((1,), (1,)), ((), ()))


def _kernel(axt, ak, av, awq, awot, bxt, bk, bv, bwq, bwot, out_hbm,
            kbuf, vbuf, wqbuf, wobuf, xtbuf, x_ref, acc_ref, outbuf,
            sem_in, sem_x, sem_out):
    s = pl.program_id(0)
    ph = s // SPP
    t = s % SPP
    slot = s % 2

    def step_copies(k_hbm, v_hbm, wq_hbm, wo_hbm, hp, sl):
        cols = pl.ds(pl.multiple_of(hp * W, W), W)
        heads = pl.ds(hp * HPS, HPS)
        return (
            pltpu.make_async_copy(wq_hbm.at[:, cols], wqbuf.at[sl], sem_in.at[0, sl]),
            pltpu.make_async_copy(k_hbm.at[:, heads], kbuf.at[sl], sem_in.at[1, sl]),
            pltpu.make_async_copy(v_hbm.at[:, heads], vbuf.at[sl], sem_in.at[2, sl]),
            pltpu.make_async_copy(wo_hbm.at[:, cols], wobuf.at[sl], sem_in.at[3, sl]),
        )

    @pl.when(s == 0)
    def _():
        pltpu.make_async_copy(axt, xtbuf, sem_x.at[0]).start()
        for cp in step_copies(ak, av, awq, awot, 0, 0):
            cp.start()
        acc_ref[...] = jnp.zeros_like(acc_ref)

    @pl.when(t == 0)
    def _():
        pltpu.make_async_copy(axt, xtbuf, sem_x.at[0]).wait()
        for b in range(B):
            x_ref[b * SQ:(b + 1) * SQ, :] = xtbuf[b].T

    for cp in step_copies(ak, av, awq, awot, 0, slot):
        cp.wait()

    nxt = s + 1
    nt = nxt % SPP

    @pl.when(nxt < SPP)
    def _():
        for cp in step_copies(ak, av, awq, awot, nt, 1 - slot):
            cp.start()

    @pl.when(jnp.logical_and(nxt >= SPP, nxt < NSTEP))
    def _():
        for cp in step_copies(bk, bv, bwq, bwot, nt, 1 - slot):
            cp.start()

    @pl.when(s == 1)
    def _():
        pltpu.make_async_copy(bxt, xtbuf, sem_x.at[0]).start()

    o_list = []
    for c in range(NC):
        rows = slice(c * CB * SQ, (c + 1) * CB * SQ)
        q = jnp.dot(x_ref[rows, :], wqbuf[slot], preferred_element_type=jnp.float32)
        q = (q * QSCALE).astype(jnp.bfloat16)
        o_rows = []
        for j in range(CB):
            b = c * CB + j
            o_heads = []
            for g in range(HPS):
                qb = q[j * SQ:(j + 1) * SQ, g * GW:(g + 1) * GW]
                q2 = jnp.concatenate([qb[:, :DH], qb[:, DH:]], axis=0)
                sc = lax.dot_general(q2, kbuf[slot, b, g], _NT,
                                     preferred_element_type=jnp.float32)
                m = jnp.max(sc, axis=-1, keepdims=True)
                p = jnp.exp2(sc - m)
                l = jnp.sum(p, axis=-1, keepdims=True)
                o2 = jnp.dot(p.astype(jnp.bfloat16), vbuf[slot, b, g],
                             preferred_element_type=jnp.float32)
                r = pl.reciprocal(l, approx=True)
                r = r * (2.0 - l * r)
                o2 = (o2 * r).astype(jnp.bfloat16)
                o_heads += [o2[:SQ], o2[SQ:]]
            o_rows.append(jnp.concatenate(o_heads, axis=1))
        o_list.append(jnp.concatenate(o_rows, axis=0))

    arow = pl.multiple_of(ph * D, 8)
    for c in range(NC):
        acc_ref[c, pl.ds(arow, D), :] += lax.dot_general(
            wobuf[slot], o_list[c], _NT, preferred_element_type=jnp.float32)

    @pl.when(s == NSTEP - 1)
    def _():
        cps = []
        for b in range(B):
            c, j = b // CB, b % CB
            rows = slice(b * SQ, (b + 1) * SQ)
            outbuf[rows, :] = acc_ref[c, :, j * SQ:(j + 1) * SQ].astype(outbuf.dtype).T
            cp = pltpu.make_async_copy(outbuf.at[rows], out_hbm.at[rows], sem_out.at[b])
            cp.start()
            cps.append(cp)
        for cp in cps:
            cp.wait()


@jax.jit
def pallas_concat_heads__gqa_block_cached__gqa_block_cached__near_ridge_kernel(
    A_x, A_k_cache, A_v_cache, A_wq, A_wo, B_x, B_k_cache, B_v_cache, B_wq, B_wo):
    axt = jnp.swapaxes(A_x, 1, 2)
    bxt = jnp.swapaxes(B_x, 1, 2)
    awot = A_wo.T
    bwot = B_wo.T
    any_spec = pl.BlockSpec(memory_space=pl.ANY)
    out = pl.pallas_call(
        _kernel,
        grid=(NSTEP,),
        in_specs=[any_spec] * 10,
        out_specs=any_spec,
        out_shape=jax.ShapeDtypeStruct((M, 2 * D), jnp.bfloat16),
        scratch_shapes=[
            pltpu.VMEM((2, B, HPS, SK, DH), jnp.bfloat16),
            pltpu.VMEM((2, B, HPS, SK, DH), jnp.bfloat16),
            pltpu.VMEM((2, D, W), jnp.bfloat16),
            pltpu.VMEM((2, D, W), jnp.bfloat16),
            pltpu.VMEM((B, D, SQ), jnp.bfloat16),
            pltpu.VMEM((M, D), jnp.bfloat16),
            pltpu.VMEM((NC, 2 * D, CB * SQ), jnp.float32),
            pltpu.VMEM((M, 2 * D), jnp.bfloat16),
            pltpu.SemaphoreType.DMA((4, 2)),
            pltpu.SemaphoreType.DMA((1,)),
            pltpu.SemaphoreType.DMA((B,)),
        ],
        compiler_params=pltpu.CompilerParams(
            dimension_semantics=("arbitrary",),
            vmem_limit_bytes=96 * 1024 * 1024,
        ),
    )(axt, A_k_cache, A_v_cache, A_wq, awot, bxt, B_k_cache, B_v_cache, B_wq, bwot)
    return out.reshape(B, SQ, 2 * D)
```
